```python
import jax
import jax.numpy as jnp

def _softmax(x, axis=-1):
    return jax.nn.softmax(x, axis=axis)
def _gelu(x):
    return jax.nn.gelu(x, approximate=True)
def _silu(x):
    return jax.nn.silu(x)
def _sigmoid(x):
    return jax.nn.sigmoid(x)
def _layernorm(x, axis=-1, eps=1e-5):
    m = jnp.mean(x, axis=axis, keepdims=True)
    v = jnp.var(x, axis=axis, keepdims=True)
    return (x - m) / jnp.sqrt(v + eps)
def _scatter_add(tgt, idx, src, axis=0):
    return tgt.at[idx].add(src)
def _segment_sum(src, seg, n):
    return jax.ops.segment_sum(src, seg, n)
class _Rng:
    def __init__(self, key):
        self._k = key
    def _next(self):
        self._k, sub = jax.random.split(self._k)
        return sub
    def normal(self, shape):
        return jax.random.normal(self._next(), shape, dtype=jnp.bfloat16)
    def randint(self, lo, hi, shape):
        return jax.random.randint(self._next(), shape, lo, hi, dtype=jnp.int32)
    def uniform(self, shape, lo=0.0, hi=1.0):
        return jax.random.uniform(self._next(), shape, jnp.bfloat16, lo, hi)
    def permutation(self, n):
        return jax.random.permutation(self._next(), n)


kernel_name = 'recurrent_scan__compressed_kv_cla__dense_activation_gelu__decode'

def setup_inputs():
    _rng = _Rng(jax.random.key(int.from_bytes(__import__("os").urandom(4), "little")))
    _w = (lambda a: (lambda t: t.astype(jnp.bfloat16) if jnp.issubdtype(t.dtype, jnp.floating) else t)(jnp.asarray(a)))
    def _A_setup():
        B, H, Sq, Sk, D, M = 2, 32, 1, 16384, 128, 512
        Dc = 4 * D
        return {
            "x": _w((lambda *s: _rng.normal(s) * 0.05)(B, Sq, M)),
            "c_kv": _w((lambda *s: _rng.normal(s) * 0.05)(B, Sk, Dc)),
            "w_q": _w((lambda *s: _rng.normal(s) * 0.05)(M, H, D) * (M ** -0.5)),
            "w_uk": _w((lambda *s: _rng.normal(s) * 0.05)(Dc, H, D) * (Dc ** -0.5)),
            "w_uv": _w((lambda *s: _rng.normal(s) * 0.05)(Dc, H, D) * (Dc ** -0.5)),
            "w_o": _w((lambda *s: _rng.normal(s) * 0.05)(H, D, M) * ((H * D) ** -0.5)),
        }
    _A_in = _A_setup()

    def _B_setup():
        B, S, D, F = 2, 1, 512, 1792
        return {
            "x": _w((lambda *s: _rng.normal(s) * 0.05)(B, S, D)),
            "w1": _w((lambda *s: _rng.normal(s) * 0.05)(D, F) * (D ** -0.5)),
            "b1": _w((lambda *s: _rng.normal(s) * 0.05)(F) * 0.01),
            "w2": _w((lambda *s: _rng.normal(s) * 0.05)(F, D) * (F ** -0.5)),
            "b2": _w((lambda *s: _rng.normal(s) * 0.05)(D) * 0.01),
        }
    _B_in = _B_setup()

    return {
        "A_x": _A_in["x"],
        "A_c_kv": _A_in["c_kv"],
        "A_w_q": _A_in["w_q"],
        "A_w_uk": _A_in["w_uk"],
        "A_w_uv": _A_in["w_uv"],
        "A_w_o": _A_in["w_o"],
        "B_x": _B_in["x"],
        "B_w1": _B_in["w1"],
        "B_b1": _B_in["b1"],
        "B_w2": _B_in["w2"],
        "B_b2": _B_in["b2"],
    }

def reference(A_x, A_c_kv, A_w_q, A_w_uk, A_w_uv, A_w_o, B_x, B_w1, B_b1, B_w2, B_b2):
    def _A_ref(x, c_kv, w_q, w_uk, w_uv, w_o):
        B, Sq, M = x.shape[0], x.shape[1], x.shape[2]
        Sk = c_kv.shape[1]
        H, D = w_q.shape[1], w_q.shape[2]
        q = jnp.einsum("bqm,mhd->bhqd", x, w_q)
        k = jnp.einsum("bkc,chd->bhkd", c_kv, w_uk)
        v = jnp.einsum("bkc,chd->bhkd", c_kv, w_uv)
        scores = jnp.einsum("bhqd,bhkd->bhqk", q, k) * (D ** -0.5)
        off = Sk - Sq
        qi = jnp.arange(Sq)[:, None]
        kj = jnp.arange(Sk)[None, :]
        cmask = kj <= (qi + off)
        scores = jnp.where(cmask[None, None], scores, -1e9)
        p = _softmax(scores, axis=-1)
        ctx = jnp.einsum("bhqk,bhkd->bhqd", p, v)
        return jnp.einsum("bhqd,hdm->bqm", ctx, w_o)

    def _B_ref(x, w1, b1, w2, b2):
        h = jnp.einsum("bsd,df->bsf", x, w1) + b1
        h = _gelu(h)
        return jnp.einsum("bsf,fd->bsd", h, w2) + b2

    x = A_x
    xn = _layernorm(x, axis=-1)
    s = _A_ref(xn, A_c_kv, A_w_q, A_w_uk, A_w_uv, A_w_o)
    g = _silu(_B_ref(xn, B_w1, B_b1, B_w2, B_b2))
    return x + s * g
```

```python
import functools

import jax
import jax.numpy as jnp
import jax.experimental.pallas as pl
import jax.experimental.pallas.tpu as pltpu

_WCH = 128
_KCH = 2048
_OCH = 4


def _kernel(x_hbm, ckv_hbm, wq_hbm, wuk_hbm, wuv_hbm, wo_hbm, w1_hbm, b1_hbm, w2_hbm, b2_hbm,
            o_hbm,
            x_v, ckv_v, wq_v, wuk_v, wuv_v, wo_v, w1_v, b1_v, w2_v, b2_v, o_v,
            wuvt_v, qabs_v, ctxc_v, sems):
    B, SK, DC = ckv_hbm.shape
    M, H, D = wq_hbm.shape
    f32, bf16 = jnp.float32, jnp.bfloat16
    n_wq, n_wc = M // _WCH, DC // _WCH
    n_k = SK // _KCH
    n_o = H // _OCH

    names = {}
    nxt = 0
    for name, n in (("x", 1), ("b1", 1), ("b2", 1), ("wq", n_wq), ("wuk", n_wc), ("wuv", n_wc),
                    ("ckv", B * n_k), ("w1", 1), ("w2", 1), ("wo", n_o), ("out", 1)):
        names[name] = nxt
        nxt += n

    def cp_small(src, dst, name):
        return pltpu.make_async_copy(src, dst, sems.at[names[name]])

    def cp_w(src, dst, name, i, rows):
        return pltpu.make_async_copy(src.at[pl.ds(i * rows, rows)], dst.at[pl.ds(i * rows, rows)],
                                     sems.at[names[name] + i])

    def cp_ckv(b, i):
        return pltpu.make_async_copy(ckv_hbm.at[b, pl.ds(i * _KCH, _KCH)],
                                     ckv_v.at[b, pl.ds(i * _KCH, _KCH)],
                                     sems.at[names["ckv"] + b * n_k + i])

    cp_small(x_hbm, x_v, "x").start()
    for i in range(n_wq):
        cp_w(wq_hbm, wq_v, "wq", i, _WCH).start()
    cp_small(b1_hbm, b1_v, "b1").start()
    cp_small(b2_hbm, b2_v, "b2").start()
    for i in range(n_wc):
        cp_w(wuk_hbm, wuk_v, "wuk", i, _WCH).start()
    for i in range(n_wc):
        cp_w(wuv_hbm, wuv_v, "wuv", i, _WCH).start()
    for b in range(B):
        for i in range(n_k):
            cp_ckv(b, i).start()
    cp_small(w1_hbm, w1_v, "w1").start()
    cp_small(w2_hbm, w2_v, "w2").start()
    for i in range(n_o):
        cp_w(wo_hbm, wo_v, "wo", i, _OCH).start()

    cp_small(x_hbm, x_v, "x").wait()
    x = x_v[...].astype(f32)
    mu = jnp.mean(x, axis=-1, keepdims=True)
    xc = x - mu
    var = jnp.mean(xc * xc, axis=-1, keepdims=True)
    xn = (xc / jnp.sqrt(var + 1e-5)).astype(bf16)

    q = [jnp.zeros((B, D), f32) for _ in range(H)]
    for i in range(n_wq):
        cp_w(wq_hbm, wq_v, "wq", i, _WCH).wait()
        wt = jnp.swapaxes(wq_v[pl.ds(i * _WCH, _WCH)], 0, 1)
        xs = xn[:, i * _WCH:(i + 1) * _WCH]
        for h in range(H):
            q[h] = q[h] + jnp.dot(xs, wt[h], preferred_element_type=f32)
    scale = D ** -0.5
    qb = [(q[h] * scale).astype(bf16) for h in range(H)]

    for i in range(n_wc):
        cp_w(wuk_hbm, wuk_v, "wuk", i, _WCH).wait()
        wt = jnp.swapaxes(wuk_v[pl.ds(i * _WCH, _WCH)], 0, 1)
        for h in range(H):
            r = jax.lax.dot_general(qb[h], wt[h], (((1,), (1,)), ((), ())),
                                    preferred_element_type=f32)
            for b in range(B):
                qabs_v[b, pl.ds(h, 1), pl.ds(i * _WCH, _WCH)] = r[b:b + 1, :]

    for i in range(n_wc):
        cp_w(wuv_hbm, wuv_v, "wuv", i, _WCH).wait()
        wuvt_v[:, pl.ds(i * _WCH, _WCH), :] = jnp.swapaxes(wuv_v[pl.ds(i * _WCH, _WCH)], 0, 1)

    for b in range(B):
        qa = qabs_v[b].astype(bf16)

        def body(i, carry, b=b, qa=qa):
            m_old, l_old, acc = carry
            cp_ckv(b, i).wait()
            c = ckv_v[b, pl.ds(pl.multiple_of(i * _KCH, _KCH), _KCH), :]
            s = jax.lax.dot_general(qa, c, (((1,), (1,)), ((), ())),
                                    preferred_element_type=f32)
            m_new = jnp.maximum(m_old, jnp.max(s, axis=-1, keepdims=True))
            alpha = jnp.exp(m_old - m_new)
            p = jnp.exp(s - m_new)
            l_new = alpha * l_old + jnp.sum(p, axis=-1, keepdims=True)
            acc = alpha * acc + jnp.dot(p.astype(bf16), c, preferred_element_type=f32)
            return m_new, l_new, acc

        init = (jnp.full((H, 1), -jnp.inf, f32), jnp.zeros((H, 1), f32), jnp.zeros((H, DC), f32))
        _, l_fin, acc = jax.lax.fori_loop(0, n_k, body, init)
        ctxc_v[b] = acc / l_fin

    cp_small(w1_hbm, w1_v, "w1").wait()
    cp_small(b1_hbm, b1_v, "b1").wait()
    b1 = b1_v[...].astype(f32)
    b1 = jnp.concatenate([b1[r:r + 1, :] for r in range(b1.shape[0])], axis=1)
    hid = jnp.dot(xn, w1_v[...], preferred_element_type=f32) + b1
    hid = jax.nn.gelu(hid, approximate=True).astype(bf16)
    cp_small(w2_hbm, w2_v, "w2").wait()
    cp_small(b2_hbm, b2_v, "b2").wait()
    b2 = b2_v[...].astype(f32)
    b2 = jnp.concatenate([b2[r:r + 1, :] for r in range(b2.shape[0])], axis=1)
    g = jnp.dot(hid, w2_v[...], preferred_element_type=f32) + b2
    g = g * jax.nn.sigmoid(g)

    out = jnp.zeros((B, M), f32)
    for i in range(n_o):
        cp_w(wo_hbm, wo_v, "wo", i, _OCH).wait()
        for h in range(i * _OCH, (i + 1) * _OCH):
            cc = ctxc_v[:, h, :].astype(bf16)
            ctx = jnp.dot(cc, wuvt_v[h], preferred_element_type=f32).astype(bf16)
            out = out + jnp.dot(ctx, wo_v[h], preferred_element_type=f32)

    o_v[...] = (x + out * g).astype(o_v.dtype)
    o_cp = cp_small(o_v, o_hbm, "out")
    o_cp.start()
    o_cp.wait()


@jax.jit
def pallas_recurrent_scan__compressed_kv_cla__dense_activation_gelu__decode_kernel(
    A_x: jax.Array,
    A_c_kv: jax.Array,
    A_w_q: jax.Array,
    A_w_uk: jax.Array,
    A_w_uv: jax.Array,
    A_w_o: jax.Array,
    B_x: jax.Array,
    B_w1: jax.Array,
    B_b1: jax.Array,
    B_w2: jax.Array,
    B_b2: jax.Array,
):
    del B_x
    B, Sq, M = A_x.shape
    _, SK, DC = A_c_kv.shape
    _, H, D = A_w_q.shape
    F = B_w1.shape[1]
    assert Sq == 1
    bf16, f32 = jnp.bfloat16, jnp.float32
    n_sems = 3 + M // _WCH + 2 * (DC // _WCH) + B * (SK // _KCH) + 2 + H // _OCH + 1

    any_spec = pl.BlockSpec(memory_space=pl.ANY)
    ins = (A_x.reshape(B, M), A_c_kv, A_w_q, A_w_uk, A_w_uv, A_w_o,
           B_w1, B_b1.reshape(F // 128, 128), B_w2, B_b2.reshape(M // 128, 128))
    out = pl.pallas_call(
        _kernel,
        out_shape=jax.ShapeDtypeStruct((B, M), A_x.dtype),
        in_specs=[any_spec] * len(ins),
        out_specs=any_spec,
        scratch_shapes=[pltpu.VMEM(a.shape, a.dtype) for a in ins] + [
            pltpu.VMEM((B, M), A_x.dtype),
            pltpu.VMEM((H, DC, D), bf16),
            pltpu.VMEM((B, H, DC), f32),
            pltpu.VMEM((B, H, DC), f32),
            pltpu.SemaphoreType.DMA((n_sems,)),
        ],
        compiler_params=pltpu.CompilerParams(vmem_limit_bytes=100 * 1024 * 1024),
    )(*ins)
    return out.reshape(B, Sq, M)
```

```python
import itertools

import jax
import jax.numpy as jnp
import jax.experimental.pallas as pl
import jax.experimental.pallas.tpu as pltpu

_WCH = 128
_KT = 2048
_KDMA = ((16384,), (8192, 8192))
_ODMA = (28, 4)


def _kernel(x_hbm, ckv_hbm, wq_hbm, wuk_hbm, wuv_hbm, wo_hbm, w1_hbm, b1_hbm, w2_hbm, b2_hbm,
            o_hbm,
            x_v, ckv_v, wq_v, wuk_v, wuv_v, wo_v, w1_v, b1_v, w2_v, b2_v, o_v,
            wuvt_v, qabs_v, ctxc_v, sems):
    B, SK, DC = ckv_hbm.shape
    M, H, D = wq_hbm.shape
    f32, bf16 = jnp.float32, jnp.bfloat16
    n_wq, n_wc = M // _WCH, DC // _WCH

    sem_id = itertools.count()
    copy = lambda src, dst: pltpu.make_async_copy(src, dst, sems.at[next(sem_id)])

    cp_x, cp_b1, cp_b2 = copy(x_hbm, x_v), copy(b1_hbm, b1_v), copy(b2_hbm, b2_v)
    cp_wq, cp_wuk, cp_wuv = copy(wq_hbm, wq_v), copy(wuk_hbm, wuk_v), copy(wuv_hbm, wuv_v)
    cp_w1, cp_w2 = copy(w1_hbm, w1_v), copy(w2_hbm, w2_v)
    cp_ckv = []
    for b in range(B):
        assert sum(_KDMA[b]) == SK
        start, chunks = 0, []
        for rows in _KDMA[b]:
            chunks.append((start, rows, copy(ckv_hbm.at[b, pl.ds(start, rows)],
                                             ckv_v.at[b, pl.ds(start, rows)])))
            start += rows
        cp_ckv.append(chunks)
    assert sum(_ODMA) == H
    cp_wo, start = [], 0
    for n in _ODMA:
        cp_wo.append((start, n, copy(wo_hbm.at[pl.ds(start, n)], wo_v.at[pl.ds(start, n)])))
        start += n
    cp_out = copy(o_v, o_hbm)

    cp_wq.start()
    cp_x.start()
    cp_wuk.start()
    cp_wuv.start()
    cp_b1.start()
    cp_b2.start()
    for b in range(B):
        for _, _, cp in cp_ckv[b]:
            cp.start()
    cp_w1.start()
    cp_w2.start()
    for _, _, cp in cp_wo:
        cp.start()

    cp_x.wait()
    x = x_v[...].astype(f32)
    mu = jnp.mean(x, axis=-1, keepdims=True)
    xc = x - mu
    var = jnp.mean(xc * xc, axis=-1, keepdims=True)
    xn = (xc / jnp.sqrt(var + 1e-5)).astype(bf16)

    q = [jnp.zeros((B, D), f32) for _ in range(H)]
    cp_wq.wait()
    for i in range(n_wq):
        wt = jnp.swapaxes(wq_v[pl.ds(i * _WCH, _WCH)], 0, 1)
        xs = xn[:, i * _WCH:(i + 1) * _WCH]
        for h in range(H):
            q[h] = q[h] + jnp.dot(xs, wt[h], preferred_element_type=f32)
    scale = D ** -0.5
    qb = [(q[h] * scale).astype(bf16) for h in range(H)]

    cp_wuk.wait()
    for i in range(n_wc):
        wt = jnp.swapaxes(wuk_v[pl.ds(i * _WCH, _WCH)], 0, 1)
        for h in range(H):
            r = jax.lax.dot_general(qb[h], wt[h], (((1,), (1,)), ((), ())),
                                    preferred_element_type=f32)
            for b in range(B):
                qabs_v[b, pl.ds(h, 1), pl.ds(i * _WCH, _WCH)] = r[b:b + 1, :]

    cp_wuv.wait()
    for i in range(n_wc):
        wuvt_v[:, pl.ds(i * _WCH, _WCH), :] = jnp.swapaxes(wuv_v[pl.ds(i * _WCH, _WCH)], 0, 1)

    for b in range(B):
        qa = qabs_v[b].astype(bf16)

        def body(i, carry, b=b, qa=qa):
            m_old, l_old, acc = carry
            c = ckv_v[b, pl.ds(pl.multiple_of(i * _KT, _KT), _KT), :]
            s = jax.lax.dot_general(qa, c, (((1,), (1,)), ((), ())),
                                    preferred_element_type=f32)
            m_new = jnp.maximum(m_old, jnp.max(s, axis=-1, keepdims=True))
            alpha = jnp.exp(m_old - m_new)
            p = jnp.exp(s - m_new)
            l_new = alpha * l_old + jnp.sum(p, axis=-1, keepdims=True)
            acc = alpha * acc + jnp.dot(p.astype(bf16), c, preferred_element_type=f32)
            return m_new, l_new, acc

        carry = (jnp.full((H, 1), -jnp.inf, f32), jnp.zeros((H, 1), f32), jnp.zeros((H, DC), f32))
        for start, rows, cp in cp_ckv[b]:
            cp.wait()
            carry = jax.lax.fori_loop(start // _KT, (start + rows) // _KT, body, carry)
        _, l_fin, acc = carry
        ctxc_v[b] = acc / l_fin

    ctx = [jnp.dot(ctxc_v[:, h, :].astype(bf16), wuvt_v[h], preferred_element_type=f32).astype(bf16)
           for h in range(H)]

    cp_w1.wait()
    cp_b1.wait()
    b1 = b1_v[...].astype(f32)
    b1 = jnp.concatenate([b1[r:r + 1, :] for r in range(b1.shape[0])], axis=1)
    hid = jnp.dot(xn, w1_v[...], preferred_element_type=f32) + b1
    hid = jax.nn.gelu(hid, approximate=True).astype(bf16)
    cp_w2.wait()
    cp_b2.wait()
    b2 = b2_v[...].astype(f32)
    b2 = jnp.concatenate([b2[r:r + 1, :] for r in range(b2.shape[0])], axis=1)
    g = jnp.dot(hid, w2_v[...], preferred_element_type=f32) + b2
    g = g * jax.nn.sigmoid(g)

    out = jnp.zeros((B, M), f32)
    for start, n, cp in cp_wo:
        cp.wait()
        for h in range(start, start + n):
            out = out + jnp.dot(ctx[h], wo_v[h], preferred_element_type=f32)

    o_v[...] = (x + out * g).astype(o_v.dtype)
    cp_out.start()
    cp_out.wait()


@jax.jit
def pallas_recurrent_scan__compressed_kv_cla__dense_activation_gelu__decode_kernel(
    A_x: jax.Array,
    A_c_kv: jax.Array,
    A_w_q: jax.Array,
    A_w_uk: jax.Array,
    A_w_uv: jax.Array,
    A_w_o: jax.Array,
    B_x: jax.Array,
    B_w1: jax.Array,
    B_b1: jax.Array,
    B_w2: jax.Array,
    B_b2: jax.Array,
):
    del B_x
    B, Sq, M = A_x.shape
    _, SK, DC = A_c_kv.shape
    _, H, D = A_w_q.shape
    F = B_w1.shape[1]
    assert Sq == 1 and F % 128 == 0 and M % 128 == 0
    bf16, f32 = jnp.bfloat16, jnp.float32
    n_sems = 9 + sum(len(c) for c in _KDMA) + len(_ODMA)

    any_spec = pl.BlockSpec(memory_space=pl.ANY)
    ins = (A_x.reshape(B, M), A_c_kv, A_w_q, A_w_uk, A_w_uv, A_w_o,
           B_w1, B_b1.reshape(F // 128, 128), B_w2, B_b2.reshape(M // 128, 128))
    out = pl.pallas_call(
        _kernel,
        out_shape=jax.ShapeDtypeStruct((B, M), A_x.dtype),
        in_specs=[any_spec] * len(ins),
        out_specs=any_spec,
        scratch_shapes=[pltpu.VMEM(a.shape, a.dtype) for a in ins] + [
            pltpu.VMEM((B, M), A_x.dtype),
            pltpu.VMEM((H, DC, D), bf16),
            pltpu.VMEM((B, H, DC), f32),
            pltpu.VMEM((B, H, DC), f32),
            pltpu.SemaphoreType.DMA((n_sems,)),
        ],
        compiler_params=pltpu.CompilerParams(vmem_limit_bytes=100 * 1024 * 1024),
    )(*ins)
    return out.reshape(B, Sq, M)
```
